```python
import jax
import jax.numpy as jnp

def _softmax(x, axis=-1):
    return jax.nn.softmax(x, axis=axis)

def _gelu(x):
    return jax.nn.gelu(x, approximate=True)

def _silu(x):
    return jax.nn.silu(x)

def _sigmoid(x):
    return jax.nn.sigmoid(x)

def _layernorm(x, axis=-1, eps=1e-05):
    m = jnp.mean(x, axis=axis, keepdims=True)
    v = jnp.var(x, axis=axis, keepdims=True)
    return (x - m) / jnp.sqrt(v + eps)

def _scatter_add(tgt, idx, src, axis=0):
    return tgt.at[idx].add(src)

def _segment_sum(src, seg, n):
    return jax.ops.segment_sum(src, seg, n)

class _Rng:

    def __init__(self, key):
        self._k = key

    def _next(self):
        self._k, sub = jax.random.split(self._k)
        return sub

    def normal(self, shape):
        return jax.random.normal(self._next(), shape, dtype=jnp.bfloat16)

    def randint(self, lo, hi, shape):
        return jax.random.randint(self._next(), shape, lo, hi, dtype=jnp.int32)

    def uniform(self, shape, lo=0.0, hi=1.0):
        return jax.random.uniform(self._next(), shape, jnp.bfloat16, lo, hi)

    def permutation(self, n):
        return jax.random.permutation(self._next(), n)
kernel_name = 'adaLN_cond__sliding_block_cached__mixer_token_mlp__decode'

def setup_inputs():
    _rng = _Rng(jax.random.key(int.from_bytes(__import__("os").urandom(4), "little")))
    _w = lambda a: (lambda t: t.astype(jnp.bfloat16) if jnp.issubdtype(t.dtype, jnp.floating) else t)(jnp.asarray(a))

    def _A_setup():
        B, Sq, D = (1, 1, 640)
        Hq, Hkv, Sk, Dh = (32, 32, 32768, 192)
        assert Hq % Hkv == 0, (Hq, Hkv)
        return {'x': _w((lambda *s: _rng.normal(s) * 0.05)(B, Sq, D)), 'k_cache': _w((lambda *s: _rng.normal(s) * 0.05)(B, Hkv, Sk, Dh)), 'v_cache': _w((lambda *s: _rng.normal(s) * 0.05)(B, Hkv, Sk, Dh)), 'wq': _w((lambda *s: _rng.normal(s) * 0.05)(D, Hq * Dh) * D ** (-0.5)), 'wo': _w((lambda *s: _rng.normal(s) * 0.05)(Hq * Dh, D) * (Hq * Dh) ** (-0.5))}
    _A_in = _A_setup()

    def _B_setup():
        B, S, D, F = (1, 1, 640, 1536)
        return {'x': _w((lambda *s: _rng.normal(s) * 0.05)(B, S, D)), 'w1': _w((lambda *s: _rng.normal(s) * 0.05)(S, F) * S ** (-0.5)), 'b1': _w((lambda *s: _rng.normal(s) * 0.05)(F) * 0.02), 'w2': _w((lambda *s: _rng.normal(s) * 0.05)(F, S) * F ** (-0.5)), 'b2': _w((lambda *s: _rng.normal(s) * 0.05)(S) * 0.02)}
    _B_in = _B_setup()
    return {'A_x': _A_in['x'], 'A_k_cache': _A_in['k_cache'], 'A_v_cache': _A_in['v_cache'], 'A_wq': _A_in['wq'], 'A_wo': _A_in['wo'], 'B_x': _B_in['x'], 'B_w1': _B_in['w1'], 'B_b1': _B_in['b1'], 'B_w2': _B_in['w2'], 'B_b2': _B_in['b2'], 'c': _w((lambda *s: _rng.normal(s) * 0.05)(1, 640)), 'w_mod': _w((lambda *s: _rng.normal(s) * 0.05)(640, 6 * 640) * 640 ** (-0.5))}

def reference(A_x, A_k_cache, A_v_cache, A_wq, A_wo, B_x, B_w1, B_b1, B_w2, B_b2, c, w_mod):

    def _A_ref(x, k_cache, v_cache, wq, wo):
        B, Sq, D = x.shape
        Hq, Dh = (32, 192)
        Hkv, Sk = (k_cache.shape[1], k_cache.shape[2])
        W = min(4096, max(256, Sk // 4))
        rep = Hq // Hkv
        q = (lambda x, *d: x.transpose(*d))((x @ wq).reshape(B, Sq, Hq, Dh), 0, 2, 1, 3)
        k = jnp.repeat(k_cache[:, :, Sk - W:, :], rep, axis=1)
        v = jnp.repeat(v_cache[:, :, Sk - W:, :], rep, axis=1)
        scores = jnp.einsum('bhqd,bhkd->bhqk', q, k) * Dh ** (-0.5)
        p = _softmax(scores, axis=-1)
        o = jnp.einsum('bhqk,bhkd->bhqd', p, v)
        return (lambda x, *d: x.transpose(*d))(o, 0, 2, 1, 3).reshape(B, Sq, Hq * Dh) @ wo

    def _B_ref(x, w1, b1, w2, b2):
        B, S, D = x.shape
        h = _layernorm(x, axis=-1)
        u = jnp.einsum('bsd,sf->bdf', h, w1) + b1
        u = _gelu(u)
        y = jnp.einsum('bdf,fs->bds', u, w2) + b2
        return (lambda x, *d: x.transpose(*d))(y, 0, 2, 1)
    x = A_x
    mod = (_silu(c) @ w_mod).reshape(c.shape[0], 6, 1, -1)
    sa, ca, ga, sb, cb, gb = (mod[:, 0].copy(), mod[:, 1].copy(), mod[:, 2].copy(), mod[:, 3].copy(), mod[:, 4].copy(), mod[:, 5].copy())
    h = _layernorm(x, axis=-1) * (1 + ca) + sa
    x = x + ga * _A_ref(h, A_k_cache, A_v_cache, A_wq, A_wo)
    h = _layernorm(x, axis=-1) * (1 + cb) + sb
    x = x + gb * _B_ref(h, B_w1, B_b1, B_w2, B_b2)
    return x
```

```python
import jax
import jax.numpy as jnp
from jax import lax
import jax.experimental.pallas as pl
import jax.experimental.pallas.tpu as pltpu

D = 640
H = 32
DH = 192
SK = 32768
W = 4096
F = 1536
PD = 3
NS = PD + 1
WQ_CH = 4
F32 = jnp.float32
BF16 = jnp.bfloat16


def _ln(x):
    m = jnp.mean(x, axis=-1, keepdims=True)
    xc = x - m
    v = jnp.mean(xc * xc, axis=-1, keepdims=True)
    return xc * lax.rsqrt(v + 1e-5)


def _kernel(x_ref, c_ref, w1_ref, b1_ref, w2_ref, b2_ref,
            kt_hbm, vt_hbm, wq_hbm, wo_hbm, wm_hbm,
            o_ref,
            kbuf, vbuf, wq_v, wobuf, wm_v, q_scr,
            ksem, vsem, wqsem, wosem, wmsem):
    def k_copy(h, slot):
        return pltpu.make_async_copy(
            kt_hbm.at[0, h, :, pl.ds(SK - W, W)], kbuf.at[slot], ksem.at[slot])

    def v_copy(h, slot):
        return pltpu.make_async_copy(
            vt_hbm.at[0, h, :, pl.ds(SK - W, W)], vbuf.at[slot], vsem.at[slot])

    def wm_copy(lo, hi, i):
        return pltpu.make_async_copy(
            wm_hbm.at[:, pl.ds(lo * D, (hi - lo) * D)],
            wm_v.at[:, pl.ds(lo * D, (hi - lo) * D)], wmsem.at[i])

    cw = H * DH // WQ_CH

    def wq_copy(i):
        return pltpu.make_async_copy(
            wq_hbm.at[:, pl.ds(i * cw, cw)], wq_v.at[:, pl.ds(i * cw, cw)], wqsem.at[i])

    def wo_copy(h, slot):
        return pltpu.make_async_copy(
            wo_hbm.at[pl.ds(pl.multiple_of(h * DH, DH), DH), :], wobuf.at[slot], wosem.at[slot])

    wm_copy(0, 2, 0).start()
    for i in range(WQ_CH):
        wq_copy(i).start()
    for h in range(PD):
        k_copy(h, h).start()
        v_copy(h, h).start()
        wo_copy(h, h).start()

    cc = c_ref[...].astype(F32)
    sc = (cc * jax.nn.sigmoid(cc)).astype(BF16)
    sc8 = jnp.broadcast_to(sc, (8, D))
    x = x_ref[0].astype(F32)

    wm_copy(0, 2, 0).wait()
    mod_a = jnp.dot(sc8, wm_v[:, 0:2 * D], preferred_element_type=F32)
    sa = mod_a[:, 0:D]
    ca = mod_a[:, D:2 * D]
    h1 = (_ln(x) * (1.0 + ca) + sa).astype(BF16)

    hpc = H // WQ_CH
    scale = DH ** -0.5
    for i in range(WQ_CH):
        wq_copy(i).wait()
        qc = jnp.dot(h1, wq_v[:, i * cw:(i + 1) * cw], preferred_element_type=F32)
        for j in range(hpc):
            q_scr[i * hpc + j] = qc[:, j * DH:(j + 1) * DH].astype(BF16)

    def head(h, acc):
        slot = h % NS
        nh = h + PD

        @pl.when(nh < H)
        def _():
            ns = nh % NS
            k_copy(nh, ns).start()
            v_copy(nh, ns).start()
            wo_copy(nh, ns).start()

        @pl.when(h == 6)
        def _():
            wm_copy(2, 5, 1).start()

        @pl.when(h == H - PD)
        def _():
            wm_copy(5, 6, 2).start()

        k_copy(h, slot).wait()
        s = jnp.dot(q_scr[h], kbuf[slot], preferred_element_type=F32) * scale
        m = jnp.max(s, axis=-1, keepdims=True)
        e = jnp.exp(s - m)
        l = jnp.sum(e, axis=-1, keepdims=True)
        v_copy(h, slot).wait()
        pv = None
        for j in range(W // 128):
            t = vbuf[slot, :, j * 128:(j + 1) * 128].astype(F32).reshape(DH // 8, 8, 128) \
                * e[:, j * 128:(j + 1) * 128][None]
            pv = t if pv is None else pv + t
        o = jnp.sum(pv, axis=-1, keepdims=True) / l[None]
        wo_copy(h, slot).wait()
        wo = wobuf[slot].astype(F32).reshape(DH // 8, 8, D)
        return acc + jnp.sum(wo * o, axis=0)

    acc = lax.fori_loop(0, H, head, jnp.zeros((8, D), F32))
    attn = jnp.sum(acc, axis=0, keepdims=True)

    wm_copy(2, 5, 1).wait()
    mod_b = jnp.dot(sc8, wm_v[:, 2 * D:5 * D], preferred_element_type=F32)[0:1]
    ga = mod_b[:, 0:D]
    sb = mod_b[:, D:2 * D]
    cb = mod_b[:, 2 * D:3 * D]
    x1 = x + ga * attn
    h2 = _ln(_ln(x1) * (1.0 + cb) + sb)
    hcol = jnp.broadcast_to(h2, (128, D)).T
    w1 = w1_ref[...].astype(F32)
    b1 = b1_ref[...].astype(F32).reshape(1, F)
    w2 = w2_ref[...].astype(F32) * 0.5
    c0 = 0.7978845608028654
    c1 = c0 * 0.044715
    yacc = None
    for j in range(F // 128):
        sl = slice(j * 128, (j + 1) * 128)
        u = hcol * w1[:, sl] + b1[:, sl]
        t = jnp.tanh(u * (c0 + c1 * (u * u)))
        g = (u * w2[:, sl]) * (1.0 + t)
        yacc = g if yacc is None else yacc + g
    y = jnp.sum(yacc.T, axis=0, keepdims=True)
    y = y + b2_ref[...].astype(F32).reshape(1, 1)
    wm_copy(5, 6, 2).wait()
    gb = jnp.dot(sc8, wm_v[:, 5 * D:6 * D], preferred_element_type=F32)[0:1]
    o_ref[0] = (x1 + gb * y).astype(o_ref.dtype)


@jax.jit
def pallas_adaLN_cond__sliding_block_cached__mixer_token_mlp__decode_kernel(
    A_x, A_k_cache, A_v_cache, A_wq, A_wo, B_x, B_w1, B_b1, B_w2, B_b2, c, w_mod,
):
    kt = jnp.swapaxes(A_k_cache, 2, 3)
    vt = jnp.swapaxes(A_v_cache, 2, 3)
    w2 = B_w2.reshape(1, F)
    vm = pl.BlockSpec(memory_space=pltpu.VMEM)
    hbm = pl.BlockSpec(memory_space=pl.ANY)
    dma = pltpu.SemaphoreType.DMA
    return pl.pallas_call(
        _kernel,
        out_shape=jax.ShapeDtypeStruct((1, 1, D), A_x.dtype),
        in_specs=[vm] * 6 + [hbm] * 5,
        out_specs=vm,
        scratch_shapes=[
            pltpu.VMEM((NS, DH, W), BF16),
            pltpu.VMEM((NS, DH, W), BF16),
            pltpu.VMEM((D, H * DH), BF16),
            pltpu.VMEM((NS, DH, D), BF16),
            pltpu.VMEM((D, 6 * D), BF16),
            pltpu.VMEM((H, 8, DH), BF16),
            dma((NS,)), dma((NS,)), dma((WQ_CH,)), dma((NS,)), dma((3,)),
        ],
        compiler_params=pltpu.CompilerParams(vmem_limit_bytes=100 * 1024 * 1024),
    )(A_x, c, B_w1, B_b1, w2, B_b2, kt, vt, A_wq, A_wo, w_mod)
```

```python
import jax
import jax.numpy as jnp
from jax import lax
import jax.experimental.pallas as pl
import jax.experimental.pallas.tpu as pltpu

D = 640
H = 32
DH = 192
SK = 32768
W = 4096
F = 1536
PD = 1
NS = PD + 1
VC = 1
VP = 0
WQ_CH = 4
F32 = jnp.float32
BF16 = jnp.bfloat16


def _ln(x):
    m = jnp.mean(x, axis=-1, keepdims=True)
    xc = x - m
    v = jnp.mean(xc * xc, axis=-1, keepdims=True)
    return xc * lax.rsqrt(v + 1e-5)


def _kernel(x_h, c_h, w1_h, b1_h, w2_h, b2_h,
            kt_hbm, vt_hbm, wq_hbm, wo_hbm, wm_hbm,
            o_ref,
            kbuf, vbuf, wq_v, wobuf, wm_v, q_scr, mb_scr,
            x_ref, c_ref, w1_ref, b1_ref, w2_ref, b2_ref,
            ksem, vsem, wqsem, wosem, wmsem, ssem):
    def k_copy(h, slot):
        return pltpu.make_async_copy(
            kt_hbm.at[0, h, :, pl.ds(SK - W, W)], kbuf.at[slot], ksem.at[slot])

    vw = W // VC

    def v_copy(h, slot, i):
        return pltpu.make_async_copy(
            vt_hbm.at[0, h, :, pl.ds(SK - W + i * vw, vw)],
            vbuf.at[slot, :, pl.ds(i * vw, vw)], vsem.at[slot * VC + i])

    def wm_copy(lo, hi, i):
        return pltpu.make_async_copy(
            wm_hbm.at[:, pl.ds(lo * D, (hi - lo) * D)],
            wm_v.at[:, pl.ds(lo * D, (hi - lo) * D)], wmsem.at[i])

    cw = H * DH // WQ_CH

    def wq_copy(i):
        return pltpu.make_async_copy(
            wq_hbm.at[:, pl.ds(i * cw, cw)], wq_v.at[:, pl.ds(i * cw, cw)], wqsem.at[i])

    def wo_copy(h, slot):
        return pltpu.make_async_copy(
            wo_hbm.at[pl.ds(pl.multiple_of(h * DH, DH), DH), :], wobuf.at[slot], wosem.at[slot])

    wm_copy(0, 2, 0).start()
    small = [pltpu.make_async_copy(a, b, ssem.at[i]) for i, (a, b) in enumerate(
        ((x_h, x_ref), (c_h, c_ref), (w1_h, w1_ref), (b1_h, b1_ref), (w2_h, w2_ref), (b2_h, b2_ref)))]
    for cp in small:
        cp.start()
    for i in range(WQ_CH):
        wq_copy(i).start()
    for h in range(PD):
        k_copy(h, h).start()
        for i in range(VC):
            v_copy(h, h, i).start(priority=VP)
        wo_copy(h, h).start()

    for cp in small:
        cp.wait()
    cc = c_ref[...].astype(F32)
    sc = (cc * jax.nn.sigmoid(cc)).astype(BF16)
    sc8 = jnp.broadcast_to(sc, (8, D))
    x = x_ref[0].astype(F32)

    wm_copy(0, 2, 0).wait()
    mod_a = jnp.dot(sc8, wm_v[:, 0:2 * D], preferred_element_type=F32)
    sa = mod_a[:, 0:D]
    ca = mod_a[:, D:2 * D]
    h1 = (_ln(x) * (1.0 + ca) + sa).astype(BF16)

    hpc = H // WQ_CH
    scale = DH ** -0.5
    for i in range(WQ_CH):
        wq_copy(i).wait()
        qc = jnp.dot(h1, wq_v[:, i * cw:(i + 1) * cw], preferred_element_type=F32)
        for j in range(hpc):
            q_scr[i * hpc + j] = qc[:, j * DH:(j + 1) * DH].astype(BF16)

    def head(h, acc):
        slot = h % NS
        nh = h + PD

        @pl.when(nh < H)
        def _():
            ns = nh % NS
            k_copy(nh, ns).start()
            for i in range(VC):
                v_copy(nh, ns, i).start(priority=VP)
            wo_copy(nh, ns).start()

        @pl.when(h == 6)
        def _():
            wm_copy(2, 5, 1).start()

        @pl.when(h == 12)
        def _():
            wm_copy(2, 5, 1).wait()
            mb_scr[...] = jnp.dot(sc8, wm_v[:, 2 * D:5 * D], preferred_element_type=F32)

        @pl.when(h == H - PD)
        def _():
            wm_copy(5, 6, 2).start()

        k_copy(h, slot).wait()
        s = jnp.dot(q_scr[h], kbuf[slot], preferred_element_type=F32) * scale
        m = jnp.max(s, axis=-1, keepdims=True)
        e = jnp.exp(s - m)
        l = jnp.sum(e, axis=-1, keepdims=True)
        pv = None
        for j in range(W // 128):
            if (j * 128) % vw == 0:
                v_copy(h, slot, j * 128 // vw).wait()
            t = vbuf[slot, :, j * 128:(j + 1) * 128].astype(F32).reshape(DH // 8, 8, 128) \
                * e[:, j * 128:(j + 1) * 128][None]
            pv = t if pv is None else pv + t
        o = jnp.sum(pv, axis=-1, keepdims=True) / l[None]
        wo_copy(h, slot).wait()
        wo = wobuf[slot].astype(F32).reshape(DH // 8, 8, D)
        return acc + jnp.sum(wo * o, axis=0)

    acc = lax.fori_loop(0, H, head, jnp.zeros((8, D), F32))
    attn = jnp.sum(acc, axis=0, keepdims=True)

    mod_b = mb_scr[0:1]
    ga = mod_b[:, 0:D]
    sb = mod_b[:, D:2 * D]
    cb = mod_b[:, 2 * D:3 * D]
    x1 = x + ga * attn
    h2 = _ln(_ln(x1) * (1.0 + cb) + sb)
    hcol = jnp.broadcast_to(h2, (128, D)).T
    w1 = w1_ref[...].astype(F32)
    b1 = b1_ref[...].astype(F32).reshape(1, F)
    w2 = w2_ref[...].astype(F32) * 0.5
    c0 = 0.7978845608028654
    c1 = c0 * 0.044715
    yacc = None
    for j in range(F // 128):
        sl = slice(j * 128, (j + 1) * 128)
        u = hcol * w1[:, sl] + b1[:, sl]
        t = jnp.tanh(u * (c0 + c1 * (u * u)))
        g = (u * w2[:, sl]) * (1.0 + t)
        yacc = g if yacc is None else yacc + g
    y = jnp.sum(yacc.T, axis=0, keepdims=True)
    y = y + b2_ref[...].astype(F32).reshape(1, 1)
    wm_copy(5, 6, 2).wait()
    gb = jnp.dot(sc8, wm_v[:, 5 * D:6 * D], preferred_element_type=F32)[0:1]
    o_ref[0] = (x1 + gb * y).astype(o_ref.dtype)


@jax.jit
def pallas_adaLN_cond__sliding_block_cached__mixer_token_mlp__decode_kernel(
    A_x, A_k_cache, A_v_cache, A_wq, A_wo, B_x, B_w1, B_b1, B_w2, B_b2, c, w_mod,
):
    kt = jnp.swapaxes(A_k_cache, 2, 3)
    vt = jnp.swapaxes(A_v_cache, 2, 3)
    w2 = B_w2.reshape(1, F)
    vm = pl.BlockSpec(memory_space=pltpu.VMEM)
    hbm = pl.BlockSpec(memory_space=pl.ANY)
    dma = pltpu.SemaphoreType.DMA
    return pl.pallas_call(
        _kernel,
        out_shape=jax.ShapeDtypeStruct((1, 1, D), A_x.dtype),
        in_specs=[hbm] * 11,
        out_specs=vm,
        scratch_shapes=[
            pltpu.VMEM((NS, DH, W), BF16),
            pltpu.VMEM((NS, DH, W), BF16),
            pltpu.VMEM((D, H * DH), BF16),
            pltpu.VMEM((NS, DH, D), BF16),
            pltpu.VMEM((D, 6 * D), BF16),
            pltpu.VMEM((H, 8, DH), BF16),
            pltpu.VMEM((8, 3 * D), F32),
            pltpu.VMEM((1, 1, D), BF16), pltpu.VMEM((1, D), BF16), pltpu.VMEM((1, F), BF16),
            pltpu.VMEM((F,), BF16), pltpu.VMEM((1, F), BF16), pltpu.VMEM((1,), BF16),
            dma((NS,)), dma((NS * VC,)), dma((WQ_CH,)), dma((NS,)), dma((3,)), dma((6,)),
        ],
        compiler_params=pltpu.CompilerParams(vmem_limit_bytes=100 * 1024 * 1024),
    )(A_x, c, B_w1, B_b1, w2, B_b2, kt, vt, A_wq, A_wo, w_mod)
```

```python
import jax
import jax.numpy as jnp
from jax import lax
import jax.experimental.pallas as pl
import jax.experimental.pallas.tpu as pltpu

D = 640
H = 32
DH = 192
SK = 32768
W = 4096
F = 1536
PD = 1
NS = PD + 1
VC = 1
VP = 0
WQ_CH = 4
TAILMODE = 0
C0 = 0.7978845608028654
C1 = C0 * 0.044715
GAM = C1 ** (1.0 / 3.0)
KC = C0 / GAM
F32 = jnp.float32
BF16 = jnp.bfloat16


def _ln(x):
    m = jnp.mean(x, axis=-1, keepdims=True)
    xc = x - m
    v = jnp.mean(xc * xc, axis=-1, keepdims=True)
    return xc * lax.rsqrt(v + 1e-5)


def _kernel(x_h, c_h, w1_h, b1_h, w2_h, b2_h,
            kt_hbm, vt_hbm, wq_hbm, wo_hbm, wm_hbm,
            o_ref,
            kbuf, vbuf, wq_v, wobuf, wm_v, q_scr, p1_scr, pb_scr, p2_scr,
            x_ref, c_ref, w1_ref, b1_ref, w2_ref, b2_ref,
            ksem, vsem, wqsem, wosem, wmsem, ssem):
    def k_copy(h, slot):
        return pltpu.make_async_copy(
            kt_hbm.at[0, h, :, pl.ds(SK - W, W)], kbuf.at[slot], ksem.at[slot])

    vw = W // VC

    def v_copy(h, slot, i):
        return pltpu.make_async_copy(
            vt_hbm.at[0, h, :, pl.ds(SK - W + i * vw, vw)],
            vbuf.at[slot, :, pl.ds(i * vw, vw)], vsem.at[slot * VC + i])

    def wm_copy(lo, hi, i):
        return pltpu.make_async_copy(
            wm_hbm.at[:, pl.ds(lo * D, (hi - lo) * D)],
            wm_v.at[:, pl.ds(lo * D, (hi - lo) * D)], wmsem.at[i])

    cw = H * DH // WQ_CH

    def wq_copy(i):
        return pltpu.make_async_copy(
            wq_hbm.at[:, pl.ds(i * cw, cw)], wq_v.at[:, pl.ds(i * cw, cw)], wqsem.at[i])

    def wo_copy(h, slot):
        return pltpu.make_async_copy(
            wo_hbm.at[pl.ds(pl.multiple_of(h * DH, DH), DH), :], wobuf.at[slot], wosem.at[slot])

    wm_copy(0, 2, 0).start()
    small = [pltpu.make_async_copy(a, b, ssem.at[i]) for i, (a, b) in enumerate(
        ((x_h, x_ref), (c_h, c_ref), (w1_h, w1_ref), (b1_h, b1_ref), (w2_h, w2_ref), (b2_h, b2_ref)))]
    for cp in small:
        cp.start()
    for i in range(WQ_CH):
        wq_copy(i).start()
    for h in range(PD):
        k_copy(h, h).start()
        for i in range(VC):
            v_copy(h, h, i).start(priority=VP)
        wo_copy(h, h).start()

    for cp in small:
        cp.wait()
    cc = c_ref[...].astype(F32)
    sc = (cc * jax.nn.sigmoid(cc)).astype(BF16)
    sc8 = jnp.broadcast_to(sc, (8, D))
    x = x_ref[0].astype(F32)

    wm_copy(0, 2, 0).wait()
    mod_a = jnp.dot(sc8, wm_v[:, 0:2 * D], preferred_element_type=F32)
    sa = mod_a[:, 0:D]
    ca = mod_a[:, D:2 * D]
    h1 = (_ln(x) * (1.0 + ca) + sa).astype(BF16)

    hpc = H // WQ_CH
    scale = DH ** -0.5
    for i in range(WQ_CH):
        wq_copy(i).wait()
        qc = jnp.dot(h1, wq_v[:, i * cw:(i + 1) * cw], preferred_element_type=F32)
        for j in range(hpc):
            q_scr[i * hpc + j] = qc[:, j * DH:(j + 1) * DH].astype(BF16)

    def head(h, acc):
        slot = h % NS
        nh = h + PD

        @pl.when(nh < H)
        def _():
            ns = nh % NS
            k_copy(nh, ns).start()
            for i in range(VC):
                v_copy(nh, ns, i).start(priority=VP)
            wo_copy(nh, ns).start()

        @pl.when(h == 1)
        def _():
            w1r = w1_ref[...].astype(F32) * GAM
            b1r = b1_ref[...].astype(F32).reshape(1, F) * GAM
            w2r = w2_ref[...].astype(F32) * (0.5 / GAM)
            p1_scr[...] = jnp.broadcast_to(w1r, (128, F)).T
            pb_scr[...] = jnp.broadcast_to(b1r, (128, F)).T
            p2_scr[...] = jnp.broadcast_to(w2r, (128, F)).T

        @pl.when(h == H - 1)
        def _():
            if TAILMODE == 0:
                wm_copy(2, 3, 1).start()
                wm_copy(3, 5, 2).start()
                wm_copy(5, 6, 3).start()

        k_copy(h, slot).wait()

        @pl.when(h == H - 1)
        def _():
            if TAILMODE == 1:
                wm_copy(2, 3, 1).start()
                wm_copy(3, 5, 2).start()
                wm_copy(5, 6, 3).start()
            if TAILMODE == 2:
                wm_copy(2, 3, 1).start()
                wm_copy(3, 5, 2).start()

        s = jnp.dot(q_scr[h], kbuf[slot], preferred_element_type=F32) * scale
        m = jnp.max(s, axis=-1, keepdims=True)
        e = jnp.exp(s - m)
        l = jnp.sum(e, axis=-1, keepdims=True)
        pv = None
        for j in range(W // 128):
            if (j * 128) % vw == 0:
                v_copy(h, slot, j * 128 // vw).wait()
            t = vbuf[slot, :, j * 128:(j + 1) * 128].astype(F32).reshape(DH // 8, 8, 128) \
                * e[:, j * 128:(j + 1) * 128][None]
            pv = t if pv is None else pv + t
        o = jnp.sum(pv, axis=-1, keepdims=True) / l[None]
        wo_copy(h, slot).wait()
        wo = wobuf[slot].astype(F32).reshape(DH // 8, 8, D)
        return acc + jnp.sum(wo * o, axis=0)

    acc = lax.fori_loop(0, H, head, jnp.zeros((8, D), F32))
    attn = jnp.sum(acc, axis=0, keepdims=True)

    if TAILMODE == 2:
        wm_copy(5, 6, 3).start()
    w1r = w1_ref[...].astype(F32)
    b1r = b1_ref[...].astype(F32).reshape(1, F)
    w2r = w2_ref[...].astype(F32) * 0.5
    s1 = jnp.sum(w1r * w2r, axis=-1, keepdims=True)
    s0 = jnp.sum(b1r * w2r, axis=-1, keepdims=True) + b2_ref[...].astype(F32).reshape(1, 1)
    wm_copy(2, 3, 1).wait()
    ga = jnp.dot(sc8, wm_v[:, 2 * D:3 * D], preferred_element_type=F32)
    x1 = x + ga * attn
    ln1 = _ln(x1)
    wm_copy(3, 5, 2).wait()
    mod_b = jnp.dot(sc8, wm_v[:, 3 * D:5 * D], preferred_element_type=F32)
    sb = mod_b[:, 0:D]
    cb = mod_b[:, D:2 * D]
    h2 = _ln(ln1 * (1.0 + cb) + sb)
    GR = 4
    accs = [None] * (D // 128)
    for g in range(F // (8 * GR)):
        rs = slice(g * 8 * GR, (g + 1) * 8 * GR)
        p1 = p1_scr[rs, :].reshape(GR, 8, 128)
        pb = pb_scr[rs, :].reshape(GR, 8, 128)
        p2 = p2_scr[rs, :].reshape(GR, 8, 128)
        for dj in range(D // 128):
            p = h2[:, dj * 128:(dj + 1) * 128][None] * p1 + pb
            t = jnp.tanh(p * (KC + p * p))
            r = jnp.sum((p * p2) * t, axis=0)
            accs[dj] = r if accs[dj] is None else accs[dj] + r
    y = jnp.sum(jnp.concatenate(accs, axis=-1), axis=0, keepdims=True)
    y = y + h2[0:1] * s1 + s0
    wm_copy(5, 6, 3).wait()
    gb = jnp.dot(sc8, wm_v[:, 5 * D:6 * D], preferred_element_type=F32)[0:1]
    o_ref[0] = (x1[0:1] + gb * y).astype(o_ref.dtype)


@jax.jit
def pallas_adaLN_cond__sliding_block_cached__mixer_token_mlp__decode_kernel(
    A_x, A_k_cache, A_v_cache, A_wq, A_wo, B_x, B_w1, B_b1, B_w2, B_b2, c, w_mod,
):
    kt = jnp.swapaxes(A_k_cache, 2, 3)
    vt = jnp.swapaxes(A_v_cache, 2, 3)
    w2 = B_w2.reshape(1, F)
    vm = pl.BlockSpec(memory_space=pltpu.VMEM)
    hbm = pl.BlockSpec(memory_space=pl.ANY)
    dma = pltpu.SemaphoreType.DMA
    return pl.pallas_call(
        _kernel,
        out_shape=jax.ShapeDtypeStruct((1, 1, D), A_x.dtype),
        in_specs=[hbm] * 11,
        out_specs=vm,
        scratch_shapes=[
            pltpu.VMEM((NS, DH, W), BF16),
            pltpu.VMEM((NS, DH, W), BF16),
            pltpu.VMEM((D, H * DH), BF16),
            pltpu.VMEM((NS, DH, D), BF16),
            pltpu.VMEM((D, 6 * D), BF16),
            pltpu.VMEM((H, 8, DH), BF16),
            pltpu.VMEM((F, 128), F32), pltpu.VMEM((F, 128), F32), pltpu.VMEM((F, 128), F32),
            pltpu.VMEM((1, 1, D), BF16), pltpu.VMEM((1, D), BF16), pltpu.VMEM((1, F), BF16),
            pltpu.VMEM((F,), BF16), pltpu.VMEM((1, F), BF16), pltpu.VMEM((1,), BF16),
            dma((NS,)), dma((NS * VC,)), dma((WQ_CH,)), dma((NS,)), dma((4,)), dma((6,)),
        ],
        compiler_params=pltpu.CompilerParams(vmem_limit_bytes=100 * 1024 * 1024),
    )(A_x, c, B_w1, B_b1, w2, B_b2, kt, vt, A_wq, A_wo, w_mod)
```

```python
import jax
import jax.numpy as jnp
from jax import lax
import jax.experimental.pallas as pl
import jax.experimental.pallas.tpu as pltpu

D = 640
H = 32
DH = 192
SK = 32768
W = 4096
F = 1536
PD = 1
NS = PD + 1
VC = 1
VP = 1
WQ_CH = 4
TAILMODE = 0
TP = 1
GBAT = 30
C0 = 0.7978845608028654
C1 = C0 * 0.044715
GAM = C1 ** (1.0 / 3.0)
KC = C0 / GAM
F32 = jnp.float32
BF16 = jnp.bfloat16


def _ln(x):
    m = jnp.mean(x, axis=-1, keepdims=True)
    xc = x - m
    v = jnp.mean(xc * xc, axis=-1, keepdims=True)
    return xc * lax.rsqrt(v + 1e-5)


def _kernel(x_h, c_h, w1_h, b1_h, w2_h, b2_h,
            kt_hbm, vt_hbm, wq_hbm, wo_hbm, wm_hbm,
            o_ref,
            kbuf, vbuf, wq_v, wobuf, wm_v, q_scr, p1_scr, pb_scr, p2_scr,
            x_ref, c_ref, w1_ref, b1_ref, w2_ref, b2_ref,
            ksem, vsem, wqsem, wosem, wmsem, ssem):
    def k_copy(h, slot):
        return pltpu.make_async_copy(
            kt_hbm.at[0, h, :, pl.ds(SK - W, W)], kbuf.at[slot], ksem.at[slot])

    vw = W // VC

    def v_copy(h, slot, i):
        return pltpu.make_async_copy(
            vt_hbm.at[0, h, :, pl.ds(SK - W + i * vw, vw)],
            vbuf.at[slot, :, pl.ds(i * vw, vw)], vsem.at[slot * VC + i])

    def wm_copy(lo, hi, i):
        return pltpu.make_async_copy(
            wm_hbm.at[:, pl.ds(lo * D, (hi - lo) * D)],
            wm_v.at[:, pl.ds(lo * D, (hi - lo) * D)], wmsem.at[i])

    cw = H * DH // WQ_CH

    def wq_copy(i):
        return pltpu.make_async_copy(
            wq_hbm.at[:, pl.ds(i * cw, cw)], wq_v.at[:, pl.ds(i * cw, cw)], wqsem.at[i])

    def wo_copy(h, slot):
        return pltpu.make_async_copy(
            wo_hbm.at[pl.ds(pl.multiple_of(h * DH, DH), DH), :], wobuf.at[slot], wosem.at[slot])

    wm_copy(0, 2, 0).start()
    small = [pltpu.make_async_copy(a, b, ssem.at[i]) for i, (a, b) in enumerate(
        ((x_h, x_ref), (c_h, c_ref), (w1_h, w1_ref), (b1_h, b1_ref), (w2_h, w2_ref), (b2_h, b2_ref)))]
    for cp in small:
        cp.start()
    for i in range(WQ_CH):
        wq_copy(i).start()
    for h in range(PD):
        k_copy(h, h).start()
        for i in range(VC):
            v_copy(h, h, i).start(priority=VP)
        wo_copy(h, h).start()

    for cp in small:
        cp.wait()
    cc = c_ref[...].astype(F32)
    sc = (cc * jax.nn.sigmoid(cc)).astype(BF16)
    sc8 = jnp.broadcast_to(sc, (8, D))
    x = x_ref[0].astype(F32)

    wm_copy(0, 2, 0).wait()
    mod_a = jnp.dot(sc8, wm_v[:, 0:2 * D], preferred_element_type=F32)
    sa = mod_a[:, 0:D]
    ca = mod_a[:, D:2 * D]
    h1 = (_ln(x) * (1.0 + ca) + sa).astype(BF16)

    hpc = H // WQ_CH
    scale = DH ** -0.5
    for i in range(WQ_CH):
        wq_copy(i).wait()
        qc = jnp.dot(h1, wq_v[:, i * cw:(i + 1) * cw], preferred_element_type=F32)
        for j in range(hpc):
            q_scr[i * hpc + j] = qc[:, j * DH:(j + 1) * DH].astype(BF16)

    def head(h, acc):
        slot = h % NS
        nh = h + PD

        @pl.when(nh < H)
        def _():
            ns = nh % NS
            k_copy(nh, ns).start()
            for i in range(VC):
                v_copy(nh, ns, i).start(priority=VP)
            wo_copy(nh, ns).start()

        @pl.when(h == 1)
        def _():
            w1r = w1_ref[...].astype(F32) * GAM
            b1r = b1_ref[...].astype(F32).reshape(1, F) * GAM
            w2r = w2_ref[...].astype(F32) * (0.5 / GAM)
            p1_scr[...] = jnp.broadcast_to(w1r, (128, F)).T
            pb_scr[...] = jnp.broadcast_to(b1r, (128, F)).T
            p2_scr[...] = jnp.broadcast_to(w2r, (128, F)).T

        @pl.when(h == H - 1)
        def _():
            if TAILMODE == 0:
                wm_copy(2, 3, 1).start(priority=TP)
                wm_copy(3, 5, 2).start(priority=TP)
                wm_copy(5, 6, 3).start(priority=TP)

        k_copy(h, slot).wait()

        @pl.when(h == H - 1)
        def _():
            if TAILMODE == 1:
                wm_copy(2, 3, 1).start(priority=TP)
                wm_copy(3, 5, 2).start(priority=TP)
                wm_copy(5, 6, 3).start(priority=TP)
            if TAILMODE == 2:
                wm_copy(2, 3, 1).start(priority=TP)
                wm_copy(3, 5, 2).start(priority=TP)

        s = jnp.dot(q_scr[h], kbuf[slot], preferred_element_type=F32) * scale
        m = jnp.max(s, axis=-1, keepdims=True)
        e = jnp.exp(s - m)
        l = jnp.sum(e, axis=-1, keepdims=True)
        pv = None
        for j in range(W // 128):
            if (j * 128) % vw == 0:
                v_copy(h, slot, j * 128 // vw).wait()
            t = vbuf[slot, :, j * 128:(j + 1) * 128].astype(F32).reshape(DH // 8, 8, 128) \
                * e[:, j * 128:(j + 1) * 128][None]
            pv = t if pv is None else pv + t
        o = jnp.sum(pv, axis=-1, keepdims=True) / l[None]
        wo_copy(h, slot).wait()
        wo = wobuf[slot].astype(F32).reshape(DH // 8, 8, D)
        return acc + jnp.sum(wo * o, axis=0)

    acc = lax.fori_loop(0, H, head, jnp.zeros((8, D), F32))
    attn = jnp.sum(acc, axis=0, keepdims=True)

    if TAILMODE == 2:
        wm_copy(5, 6, 3).start(priority=TP)
    w1r = w1_ref[...].astype(F32)
    b1r = b1_ref[...].astype(F32).reshape(1, F)
    w2r = w2_ref[...].astype(F32) * 0.5
    s1 = jnp.sum(w1r * w2r, axis=-1, keepdims=True)
    s0 = jnp.sum(b1r * w2r, axis=-1, keepdims=True) + b2_ref[...].astype(F32).reshape(1, 1)
    wm_copy(2, 3, 1).wait()
    ga = jnp.dot(sc8, wm_v[:, 2 * D:3 * D], preferred_element_type=F32)
    x1 = x + ga * attn
    ln1 = _ln(x1)
    wm_copy(3, 5, 2).wait()
    mod_b = jnp.dot(sc8, wm_v[:, 3 * D:5 * D], preferred_element_type=F32)
    sb = mod_b[:, 0:D]
    cb = mod_b[:, D:2 * D]
    h2 = _ln(ln1 * (1.0 + cb) + sb)

    def gb_dot():
        wm_copy(5, 6, 3).wait()
        return jnp.dot(sc8, wm_v[:, 5 * D:6 * D], preferred_element_type=F32)[0:1]

    GR = 4
    accs = [None] * (D // 128)
    for g in range(F // (8 * GR)):
        if g == GBAT:
            gb = gb_dot()
        rs = slice(g * 8 * GR, (g + 1) * 8 * GR)
        p1 = p1_scr[rs, :].reshape(GR, 8, 128)
        pb = pb_scr[rs, :].reshape(GR, 8, 128)
        p2 = p2_scr[rs, :].reshape(GR, 8, 128)
        for dj in range(D // 128):
            p = h2[:, dj * 128:(dj + 1) * 128][None] * p1 + pb
            t = jnp.tanh(p * (KC + p * p))
            r = jnp.sum((p * p2) * t, axis=0)
            accs[dj] = r if accs[dj] is None else accs[dj] + r
    y = jnp.sum(jnp.concatenate(accs, axis=-1), axis=0, keepdims=True)
    y = y + h2[0:1] * s1 + s0
    if GBAT >= F // (8 * GR):
        gb = gb_dot()
    o_ref[0] = (x1[0:1] + gb * y).astype(o_ref.dtype)


@jax.jit
def pallas_adaLN_cond__sliding_block_cached__mixer_token_mlp__decode_kernel(
    A_x, A_k_cache, A_v_cache, A_wq, A_wo, B_x, B_w1, B_b1, B_w2, B_b2, c, w_mod,
):
    kt = jnp.swapaxes(A_k_cache, 2, 3)
    vt = jnp.swapaxes(A_v_cache, 2, 3)
    w2 = B_w2.reshape(1, F)
    vm = pl.BlockSpec(memory_space=pltpu.VMEM)
    hbm = pl.BlockSpec(memory_space=pl.ANY)
    dma = pltpu.SemaphoreType.DMA
    return pl.pallas_call(
        _kernel,
        out_shape=jax.ShapeDtypeStruct((1, 1, D), A_x.dtype),
        in_specs=[hbm] * 11,
        out_specs=vm,
        scratch_shapes=[
            pltpu.VMEM((NS, DH, W), BF16),
            pltpu.VMEM((NS, DH, W), BF16),
            pltpu.VMEM((D, H * DH), BF16),
            pltpu.VMEM((NS, DH, D), BF16),
            pltpu.VMEM((D, 6 * D), BF16),
            pltpu.VMEM((H, 8, DH), BF16),
            pltpu.VMEM((F, 128), F32), pltpu.VMEM((F, 128), F32), pltpu.VMEM((F, 128), F32),
            pltpu.VMEM((1, 1, D), BF16), pltpu.VMEM((1, D), BF16), pltpu.VMEM((1, F), BF16),
            pltpu.VMEM((F,), BF16), pltpu.VMEM((1, F), BF16), pltpu.VMEM((1,), BF16),
            dma((NS,)), dma((NS * VC,)), dma((WQ_CH,)), dma((NS,)), dma((4,)), dma((6,)),
        ],
        compiler_params=pltpu.CompilerParams(vmem_limit_bytes=100 * 1024 * 1024),
    )(A_x, c, B_w1, B_b1, w2, B_b2, kt, vt, A_wq, A_wo, w_mod)
```

```python
import jax
import jax.numpy as jnp
from jax import lax
import jax.experimental.pallas as pl
import jax.experimental.pallas.tpu as pltpu

D = 640
H = 32
DH = 192
SK = 32768
W = min(4096, max(256, SK // 4))
F = 1536
PD = 1
NS = PD + 1
WQ_CH = 4
GBAT = 30
C0 = 0.7978845608028654
C1 = C0 * 0.044715
GAM = C1 ** (1.0 / 3.0)
KC = C0 / GAM
F32 = jnp.float32
BF16 = jnp.bfloat16


def _ln(x):
    m = jnp.mean(x, axis=-1, keepdims=True)
    xc = x - m
    v = jnp.mean(xc * xc, axis=-1, keepdims=True)
    return xc * lax.rsqrt(v + 1e-5)


def _kernel(x_h, c_h, w1_h, b1_h, w2_h, b2_h,
            kt_hbm, vt_hbm, wq_hbm, wo_hbm, wm_hbm,
            o_ref,
            kbuf, vbuf, wq_v, wobuf, wm_v, q_scr, p1_scr, pb_scr, p2_scr,
            x_ref, c_ref, w1_ref, b1_ref, w2_ref, b2_ref,
            ksem, vsem, wqsem, wosem, wmsem, ssem):
    def k_copy(h, slot):
        return pltpu.make_async_copy(
            kt_hbm.at[0, h, :, pl.ds(SK - W, W)], kbuf.at[slot], ksem.at[slot])

    def v_copy(h, slot):
        return pltpu.make_async_copy(
            vt_hbm.at[0, h, :, pl.ds(SK - W, W)], vbuf.at[slot], vsem.at[slot])

    def wm_copy(lo, hi, i):
        return pltpu.make_async_copy(
            wm_hbm.at[:, pl.ds(lo * D, (hi - lo) * D)],
            wm_v.at[:, pl.ds(lo * D, (hi - lo) * D)], wmsem.at[i])

    cw = H * DH // WQ_CH

    def wq_copy(i):
        return pltpu.make_async_copy(
            wq_hbm.at[:, pl.ds(i * cw, cw)], wq_v.at[:, pl.ds(i * cw, cw)], wqsem.at[i])

    def wo_copy(h, slot):
        return pltpu.make_async_copy(
            wo_hbm.at[pl.ds(pl.multiple_of(h * DH, DH), DH), :], wobuf.at[slot], wosem.at[slot])

    wm_copy(0, 2, 0).start()
    small = [pltpu.make_async_copy(a, b, ssem.at[i]) for i, (a, b) in enumerate(
        ((x_h, x_ref), (c_h, c_ref), (w1_h, w1_ref), (b1_h, b1_ref), (w2_h, w2_ref), (b2_h, b2_ref)))]
    for cp in small:
        cp.start()
    for i in range(WQ_CH):
        wq_copy(i).start()
    for h in range(PD):
        k_copy(h, h).start()
        v_copy(h, h).start(priority=1)
        wo_copy(h, h).start()

    for cp in small:
        cp.wait()
    cc = c_ref[...].astype(F32)
    sc = (cc * jax.nn.sigmoid(cc)).astype(BF16)
    sc8 = jnp.broadcast_to(sc, (8, D))
    x = x_ref[0].astype(F32)

    wm_copy(0, 2, 0).wait()
    mod_a = jnp.dot(sc8, wm_v[:, 0:2 * D], preferred_element_type=F32)
    sa = mod_a[:, 0:D]
    ca = mod_a[:, D:2 * D]
    h1 = (_ln(x) * (1.0 + ca) + sa).astype(BF16)

    hpc = H // WQ_CH
    scale = DH ** -0.5
    for i in range(WQ_CH):
        wq_copy(i).wait()
        qc = jnp.dot(h1, wq_v[:, i * cw:(i + 1) * cw], preferred_element_type=F32)
        for j in range(hpc):
            q_scr[i * hpc + j] = qc[:, j * DH:(j + 1) * DH].astype(BF16)

    def head(h, acc):
        slot = h % NS
        nh = h + PD

        @pl.when(nh < H)
        def _():
            ns = nh % NS
            k_copy(nh, ns).start()
            v_copy(nh, ns).start(priority=1)
            wo_copy(nh, ns).start()

        @pl.when(h == 1)
        def _():
            w1r = w1_ref[...].astype(F32) * GAM
            b1r = b1_ref[...].astype(F32).reshape(1, F) * GAM
            w2r = w2_ref[...].astype(F32) * (0.5 / GAM)
            p1_scr[...] = jnp.broadcast_to(w1r, (128, F)).T
            pb_scr[...] = jnp.broadcast_to(b1r, (128, F)).T
            p2_scr[...] = jnp.broadcast_to(w2r, (128, F)).T

        @pl.when(h == H - 1)
        def _():
            wm_copy(2, 3, 1).start(priority=1)
            wm_copy(3, 5, 2).start(priority=1)
            wm_copy(5, 6, 3).start(priority=1)

        k_copy(h, slot).wait()
        s = jnp.dot(q_scr[h], kbuf[slot], preferred_element_type=F32) * scale
        m = jnp.max(s, axis=-1, keepdims=True)
        e = jnp.exp(s - m)
        l = jnp.sum(e, axis=-1, keepdims=True)
        v_copy(h, slot).wait()
        pv = None
        for j in range(W // 128):
            t = vbuf[slot, :, j * 128:(j + 1) * 128].astype(F32).reshape(DH // 8, 8, 128) \
                * e[:, j * 128:(j + 1) * 128][None]
            pv = t if pv is None else pv + t
        o = jnp.sum(pv, axis=-1, keepdims=True) / l[None]
        wo_copy(h, slot).wait()
        wo = wobuf[slot].astype(F32).reshape(DH // 8, 8, D)
        return acc + jnp.sum(wo * o, axis=0)

    acc = lax.fori_loop(0, H, head, jnp.zeros((8, D), F32))
    attn = jnp.sum(acc, axis=0, keepdims=True)

    w1r = w1_ref[...].astype(F32)
    b1r = b1_ref[...].astype(F32).reshape(1, F)
    w2r = w2_ref[...].astype(F32) * 0.5
    s1 = jnp.sum(w1r * w2r, axis=-1, keepdims=True)
    s0 = jnp.sum(b1r * w2r, axis=-1, keepdims=True) + b2_ref[...].astype(F32).reshape(1, 1)
    wm_copy(2, 3, 1).wait()
    ga = jnp.dot(sc8, wm_v[:, 2 * D:3 * D], preferred_element_type=F32)
    x1 = x + ga * attn
    ln1 = _ln(x1)
    wm_copy(3, 5, 2).wait()
    mod_b = jnp.dot(sc8, wm_v[:, 3 * D:5 * D], preferred_element_type=F32)
    sb = mod_b[:, 0:D]
    cb = mod_b[:, D:2 * D]
    h2 = _ln(ln1 * (1.0 + cb) + sb)

    def gb_dot():
        wm_copy(5, 6, 3).wait()
        return jnp.dot(sc8, wm_v[:, 5 * D:6 * D], preferred_element_type=F32)[0:1]

    GR = 4
    accs = [None] * (D // 128)
    for g in range(F // (8 * GR)):
        if g == GBAT:
            gb = gb_dot()
        rs = slice(g * 8 * GR, (g + 1) * 8 * GR)
        p1 = p1_scr[rs, :].reshape(GR, 8, 128)
        pb = pb_scr[rs, :].reshape(GR, 8, 128)
        p2 = p2_scr[rs, :].reshape(GR, 8, 128)
        for dj in range(D // 128):
            p = h2[:, dj * 128:(dj + 1) * 128][None] * p1 + pb
            t = jnp.tanh(p * (KC + p * p))
            r = jnp.sum((p * p2) * t, axis=0)
            accs[dj] = r if accs[dj] is None else accs[dj] + r
    y = jnp.sum(jnp.concatenate(accs, axis=-1), axis=0, keepdims=True)
    y = y + h2[0:1] * s1 + s0
    o_ref[0] = (x1[0:1] + gb * y).astype(o_ref.dtype)


@jax.jit
def pallas_adaLN_cond__sliding_block_cached__mixer_token_mlp__decode_kernel(
    A_x, A_k_cache, A_v_cache, A_wq, A_wo, B_x, B_w1, B_b1, B_w2, B_b2, c, w_mod,
):
    kt = jnp.swapaxes(A_k_cache, 2, 3)
    vt = jnp.swapaxes(A_v_cache, 2, 3)
    w2 = B_w2.reshape(1, F)
    vm = pl.BlockSpec(memory_space=pltpu.VMEM)
    hbm = pl.BlockSpec(memory_space=pl.ANY)
    dma = pltpu.SemaphoreType.DMA
    return pl.pallas_call(
        _kernel,
        out_shape=jax.ShapeDtypeStruct((1, 1, D), A_x.dtype),
        in_specs=[hbm] * 11,
        out_specs=vm,
        scratch_shapes=[
            pltpu.VMEM((NS, DH, W), BF16),
            pltpu.VMEM((NS, DH, W), BF16),
            pltpu.VMEM((D, H * DH), BF16),
            pltpu.VMEM((NS, DH, D), BF16),
            pltpu.VMEM((D, 6 * D), BF16),
            pltpu.VMEM((H, 8, DH), BF16),
            pltpu.VMEM((F, 128), F32), pltpu.VMEM((F, 128), F32), pltpu.VMEM((F, 128), F32),
            pltpu.VMEM((1, 1, D), BF16), pltpu.VMEM((1, D), BF16), pltpu.VMEM((1, F), BF16),
            pltpu.VMEM((F,), BF16), pltpu.VMEM((1, F), BF16), pltpu.VMEM((1,), BF16),
            dma((NS,)), dma((NS,)), dma((WQ_CH,)), dma((NS,)), dma((4,)), dma((6,)),
        ],
        compiler_params=pltpu.CompilerParams(vmem_limit_bytes=100 * 1024 * 1024),
    )(A_x, c, B_w1, B_b1, w2, B_b2, kt, vt, A_wq, A_wo, w_mod)
```
